```python
import os as _os
_os.environ.setdefault("JAX_PLATFORMS", "cpu")
import jax
import jax.numpy as jnp

def _softmax(x, axis=-1):
    return jax.nn.softmax(x, axis=axis)
def _gelu(x):
    return jax.nn.gelu(x, approximate=True)
def _silu(x):
    return jax.nn.silu(x)
def _sigmoid(x):
    return jax.nn.sigmoid(x)
def _layernorm(x, axis=-1, eps=1e-5):
    m = jnp.mean(x, axis=axis, keepdims=True)
    v = jnp.var(x, axis=axis, keepdims=True)
    return (x - m) / jnp.sqrt(v + eps)
def _scatter_add(tgt, idx, src, axis=0):
    return tgt.at[idx].add(src)
def _segment_sum(src, seg, n):
    return jax.ops.segment_sum(src, seg, n)
class _Rng:
    def __init__(self, key):
        self._k = key
    def _next(self):
        self._k, sub = jax.random.split(self._k)
        return sub
    def normal(self, shape):
        return jax.random.normal(self._next(), shape, dtype=jnp.bfloat16)
    def randint(self, lo, hi, shape):
        return jax.random.randint(self._next(), shape, lo, hi, dtype=jnp.int32)
    def uniform(self, shape, lo=0.0, hi=1.0):
        return jax.random.uniform(self._next(), shape, jnp.bfloat16, lo, hi)
    def permutation(self, n):
        return jax.random.permutation(self._next(), n)


kernel_name = 'concat_heads__gqa_block_cached__sliding_block_cached__decode'

def setup_inputs():
    _rng = _Rng(jax.random.key(int.from_bytes(__import__("os").urandom(4), "little")))
    _w = (lambda a: (lambda t: t.astype(jnp.bfloat16) if jnp.issubdtype(t.dtype, jnp.floating) else t)(jnp.asarray(a)))
    def _A_setup():
        B, Sq, D = 2, 1, 448
        Hq, Hkv, Sk, Dh = 16, 8, 8192, 256
        assert Hq % Hkv == 0, (Hq, Hkv)
        return {
            "x": _w((lambda *s: _rng.normal(s) * 0.8)(B, Sq, D)),
            "k_cache": _w((lambda *s: _rng.normal(s) * 0.8)(B, Hkv, Sk, Dh)),
            "v_cache": _w((lambda *s: _rng.normal(s) * 0.05)(B, Hkv, Sk, Dh)),
            "wq": _w((lambda *s: _rng.normal(s) * 0.8)(D, Hq * Dh) * (D ** -0.5)),
            "wo": _w((lambda *s: _rng.normal(s) * 0.05)(Hq * Dh, D) * ((Hq * Dh) ** -0.5)),
        }
    _A_in = _A_setup()

    def _B_setup():
        B, Sq, D = 2, 1, 448
        Hq, Hkv, Sk, Dh = 16, 8, 8192, 256
        assert Hq % Hkv == 0, (Hq, Hkv)
        return {
            "x": _w((lambda *s: _rng.normal(s) * 0.8)(B, Sq, D)),
            "k_cache": _w((lambda *s: _rng.normal(s) * 0.8)(B, Hkv, Sk, Dh)),
            "v_cache": _w((lambda *s: _rng.normal(s) * 0.05)(B, Hkv, Sk, Dh)),
            "wq": _w((lambda *s: _rng.normal(s) * 0.8)(D, Hq * Dh) * (D ** -0.5)),
            "wo": _w((lambda *s: _rng.normal(s) * 0.05)(Hq * Dh, D) * ((Hq * Dh) ** -0.5)),
        }
    _B_in = _B_setup()

    return {
        "A_x": _A_in["x"],
        "A_k_cache": _A_in["k_cache"],
        "A_v_cache": _A_in["v_cache"],
        "A_wq": _A_in["wq"],
        "A_wo": _A_in["wo"],
        "B_x": _B_in["x"],
        "B_k_cache": _B_in["k_cache"],
        "B_v_cache": _B_in["v_cache"],
        "B_wq": _B_in["wq"],
        "B_wo": _B_in["wo"],
    }

def reference(A_x, A_k_cache, A_v_cache, A_wq, A_wo, B_x, B_k_cache, B_v_cache, B_wq, B_wo):
    def _A_ref(x, k_cache, v_cache, wq, wo):
        B, Sq, D = x.shape
        Hq, Dh = 16, 256
        Hkv = k_cache.shape[1]
        rep = Hq // Hkv
        q = (lambda x, *d: x.transpose(*d))((x @ wq).reshape(B, Sq, Hq, Dh), 0, 2, 1, 3)
        k = jnp.repeat(k_cache, rep, axis=1)
        v = jnp.repeat(v_cache, rep, axis=1)
        scores = jnp.einsum("bhqd,bhkd->bhqk", q, k) * (Dh ** -0.5)
        p = _softmax(scores, axis=-1)
        o = jnp.einsum("bhqk,bhkd->bhqd", p, v)
        return (lambda x, *d: x.transpose(*d))(o, 0, 2, 1, 3).reshape(B, Sq, Hq * Dh) @ wo

    def _B_ref(x, k_cache, v_cache, wq, wo):
        B, Sq, D = x.shape
        Hq, Dh = 16, 256
        Hkv, Sk = k_cache.shape[1], k_cache.shape[2]
        W = min(4096, max(256, Sk // 4))
        rep = Hq // Hkv
        q = (lambda x, *d: x.transpose(*d))((x @ wq).reshape(B, Sq, Hq, Dh), 0, 2, 1, 3)
        k = jnp.repeat(k_cache[:, :, Sk - W:, :], rep, axis=1)
        v = jnp.repeat(v_cache[:, :, Sk - W:, :], rep, axis=1)
        scores = jnp.einsum("bhqd,bhkd->bhqk", q, k) * (Dh ** -0.5)
        p = _softmax(scores, axis=-1)
        o = jnp.einsum("bhqk,bhkd->bhqd", p, v)
        return (lambda x, *d: x.transpose(*d))(o, 0, 2, 1, 3).reshape(B, Sq, Hq * Dh) @ wo

    a = _A_ref(A_x, A_k_cache, A_v_cache, A_wq, A_wo)
    b = _B_ref(B_x, B_k_cache, B_v_cache, B_wq, B_wo)
    return jnp.concatenate([a, b], axis=-1)
```

```python
import functools
import numpy as np
import jax
import jax.numpy as jnp
from jax import lax
from jax.experimental import pallas as pl
from jax.experimental.pallas import tpu as pltpu

B, D, HQ, HKV, SK, DH = 2, 448, 16, 8, 8192, 256
W = min(4096, max(256, SK // 4))
REP = HQ // HKV
HW = REP * DH


def make(G=2048, NG=4, ROWS=64, WROWS=32, prios=(0, 1), compute=True):
    NCA, NCB = SK // G, W // G
    NA = HKV * B * NCA
    NSTEP = NA + HKV * B * NCB
    NEG = float(np.finfo(np.float32).min)

    def kern(xa, ka, va, wqa, woa, xb, kb, vb, wqb, wob, o_ref,
             xbuf, wqbuf, wobuf, kvbuf, xsem, wsem, kvsem):
        def issue_from(j, slot, k, v, wq, wo, nc, off, tbase):
            h = j // (B * nc)
            b = (j // nc) % B
            c = j % nc
            t = tbase + h
            col = pl.multiple_of(h * HW, HW)

            @pl.when(jnp.logical_and(b == 0, c == 0))
            def _():
                for r in range(D // WROWS):
                    pltpu.make_async_copy(wq.at[pl.ds(r * WROWS, WROWS), pl.ds(col, HW)],
                                          wqbuf.at[t, pl.ds(r * WROWS, WROWS), :],
                                          wsem.at[0, t]).start(priority=prios[r % len(prios)])
            row0 = pl.multiple_of(off + c * G, G)
            n = 0
            for r in range(G // ROWS):
                for a, src in enumerate((k, v)):
                    pltpu.make_async_copy(src.at[b, h, pl.ds(row0 + r * ROWS, ROWS), :],
                                          kvbuf.at[slot, a, pl.ds(r * ROWS, ROWS), :],
                                          kvsem.at[slot, a]).start(priority=prios[n % len(prios)])
                    n += 1

            @pl.when(jnp.logical_and(b == B - 1, c == nc - 1))
            def _():
                for r in range(D // WROWS):
                    pltpu.make_async_copy(wo.at[pl.ds(r * WROWS, WROWS), pl.ds(col, HW)],
                                          wobuf.at[t, pl.ds(r * WROWS, WROWS), :],
                                          wsem.at[1, t]).start(priority=prios[r % len(prios)])

        def issue(step):
            slot = step % NG

            @pl.when(step < NA)
            def _():
                issue_from(step, slot, ka, va, wqa, woa, NCA, 0, 0)

            @pl.when(jnp.logical_and(step >= NA, step < NSTEP))
            def _():
                issue_from(step - NA, slot, kb, vb, wqb, wob, NCB, SK - W, HKV)

        xcp = [pltpu.make_async_copy(x, xbuf.at[i], xsem.at[i]) for i, x in enumerate((xa, xb))]
        for cp in xcp:
            cp.start()

        def pro(s, c):
            issue_from(s, s, ka, va, wqa, woa, NCA, 0, 0)
            return c
        lax.fori_loop(0, NG, pro, 0)
        for cp in xcp:
            cp.wait()

        row = lax.broadcasted_iota(jnp.int32, (8, DH), 0)
        even = (row % 2) == 0

        def branch(br, nc, base):
            xf = xbuf[br].astype(jnp.float32)
            x16 = jnp.concatenate([jnp.broadcast_to(xf[0:1], (8, D)),
                                   jnp.broadcast_to(xf[1:2], (8, D))], axis=0).astype(jnp.bfloat16)

            def head(h, oacc):
                t = br * HKV + h
                pltpu.make_async_copy(wqbuf.at[t], wqbuf.at[t], wsem.at[0, t]).wait()
                q16 = jnp.dot(x16, wqbuf[t], preferred_element_type=jnp.float32)
                outs = []
                for b in range(B):
                    qb = q16[8 * b:8 * b + 8]
                    q8 = jnp.where(even, qb[:, :DH], qb[:, DH:]).astype(jnp.bfloat16)

                    def chunk(c, carry):
                        m, l, acc = carry
                        step = base + (h * B + b) * nc + c
                        slot = step % NG
                        pltpu.make_async_copy(kvbuf.at[slot, 0], kvbuf.at[slot, 0], kvsem.at[slot, 0]).wait()
                        if compute:
                            s = lax.dot_general(q8, kvbuf[slot, 0], (((1,), (1,)), ((), ())),
                                                preferred_element_type=jnp.float32) * (DH ** -0.5)
                            m_new = jnp.maximum(m, jnp.max(s, axis=1, keepdims=True))
                            alpha = jnp.exp(m - m_new)
                            p = jnp.exp(s - m_new)
                            l = alpha * l + jnp.sum(p, axis=1, keepdims=True)
                        pltpu.make_async_copy(kvbuf.at[slot, 1], kvbuf.at[slot, 1], kvsem.at[slot, 1]).wait()
                        if compute:
                            acc = alpha * acc + jnp.dot(p.astype(jnp.bfloat16), kvbuf[slot, 1],
                                                        preferred_element_type=jnp.float32)
                            m = m_new
                        issue(step + NG)
                        return m, l, acc

                    m, l, acc = lax.fori_loop(
                        0, nc, chunk,
                        (jnp.full((8, 1), NEG, jnp.float32), jnp.zeros((8, 1), jnp.float32),
                         jnp.zeros((8, DH), jnp.float32)))
                    o8 = acc / l
                    outs.append(jnp.concatenate([jnp.where(even, o8, 0.0), jnp.where(even, 0.0, o8)], axis=1))
                o16 = jnp.concatenate(outs, axis=0).astype(jnp.bfloat16)
                pltpu.make_async_copy(wobuf.at[t], wobuf.at[t], wsem.at[1, t]).wait()
                return oacc + lax.dot_general(o16, wobuf[t], (((1,), (1,)), ((), ())),
                                              preferred_element_type=jnp.float32)

            oacc = lax.fori_loop(0, HKV, head, jnp.zeros((16, D), jnp.float32))
            return jnp.concatenate([oacc[0:1] + oacc[1:2], oacc[8:9] + oacc[9:10]], axis=0)

        ra = branch(0, NCA, 0)
        rb = branch(1, NCB, NA)
        o_ref[...] = jnp.concatenate([ra, rb], axis=1).astype(o_ref.dtype)

    @jax.jit
    def f(A_x, A_k_cache, A_v_cache, A_wq, A_wo, B_x, B_k_cache, B_v_cache, B_wq, B_wo):
        out = pl.pallas_call(
            kern,
            in_specs=[pl.BlockSpec(memory_space=pltpu.HBM)] * 10,
            out_specs=pl.BlockSpec(memory_space=pltpu.VMEM),
            out_shape=jax.ShapeDtypeStruct((B, 2 * D), jnp.bfloat16),
            scratch_shapes=[
                pltpu.VMEM((2, B, D), jnp.bfloat16),
                pltpu.VMEM((2 * HKV, D, HW), jnp.bfloat16),
                pltpu.VMEM((2 * HKV, D, HW), jnp.bfloat16),
                pltpu.VMEM((NG, 2, G, DH), jnp.bfloat16),
                pltpu.SemaphoreType.DMA((2,)),
                pltpu.SemaphoreType.DMA((2, 2 * HKV)),
                pltpu.SemaphoreType.DMA((NG, 2)),
            ],
            compiler_params=pltpu.CompilerParams(vmem_limit_bytes=100 * 1024 * 1024),
        )(A_x.reshape(B, D), A_k_cache, A_v_cache, A_wq, A_wo.T,
          B_x.reshape(B, D), B_k_cache, B_v_cache, B_wq, B_wo.T)
        return out.reshape(B, 1, 2 * D)
    return f


_impl = make()


@jax.jit
def pallas_concat_heads__gqa_block_cached__sliding_block_cached__decode_kernel(
    A_x, A_k_cache, A_v_cache, A_wq, A_wo, B_x, B_k_cache, B_v_cache, B_wq, B_wo
):
    return _impl(A_x, A_k_cache, A_v_cache, A_wq, A_wo, B_x, B_k_cache, B_v_cache, B_wq, B_wo)
```

```python
import functools
import numpy as np
import jax
import jax.numpy as jnp
from jax import lax
from jax.experimental import pallas as pl
from jax.experimental.pallas import tpu as pltpu

B, D, HQ, HKV, SK, DH = 2, 448, 16, 8, 8192, 256
W = min(4096, max(256, SK // 4))
REP = HQ // HKV
HW = REP * DH
HD = HQ * DH

PC = ((0, 0, 64, 0), (1, 0, 64, 1), (0, 64, 128, 1), (1, 64, 128, 0), (0, 192, 64, 0), (1, 192, 64, 1))
PS = ((0, 0, 64, 0), (1, 0, 64, 1), (1, 64, 64, 0), (0, 64, 64, 1), (1, 128, 64, 0), (0, 128, 64, 1), (0, 192, 64, 0), (1, 192, 64, 1))
PS2 = ((0, 0, 64, 0), (1, 0, 64, 1), (0, 64, 64, 1), (1, 64, 64, 0), (0, 128, 64, 1), (1, 128, 64, 0), (0, 192, 64, 0), (1, 192, 64, 1))
PATS = dict(PC=PC, PS=PS, PS2=PS2)


def make(G=1024, NG=4, pat='PC', wpat='PS', nobc=True, NP=4, xp=(0, 0)):
    NCA, NCB = SK // G, W // G
    NA = HKV * B * NCA
    NSTEP = NA + HKV * B * NCB
    NEG = float(np.finfo(np.float32).min)
    SEQ = PATS[pat]
    WSEQ = PATS[wpat]
    NWIN = D // 16
    NOB = 2 * D // 128
    assert NP <= NG and NWIN % NP == 0

    def kern(xa, ka, va, wqa, woa, xb, kb, vb, wqb, wob, o_ref,
             xbuf, wqbuf, wobuf, kvbuf, qbuf, obuf, xsem, wqsem, wosem, kvsem):
        def w_pair(srcs, srows, dsts, drows, sems):
            for (a, o, _, p) in WSEQ:
                u = o // 64
                r, c = 8 * (u // 2), (HD // 2) * (u % 2)
                pltpu.make_async_copy(srcs[a].at[pl.ds(srows[a] + r, 8), pl.ds(c, HD // 2)],
                                      dsts[a].at[pl.ds(drows[a] + r, 8), pl.ds(c, HD // 2)],
                                      sems[a]).start(priority=p)

        def issue_kv(j, slot, k, v, nc, off):
            seg = j // nc
            b, h = seg // HKV, seg % HKV
            row0 = pl.multiple_of(off + (j % nc) * G, G)
            for w in range(0, G, 256):
                for (a, o, n, p) in SEQ:
                    pltpu.make_async_copy((k, v)[a].at[b, h, pl.ds(row0 + w + o, n), :],
                                          kvbuf.at[slot, a, pl.ds(w + o, n), :],
                                          kvsem.at[slot, a]).start(priority=p)

        def issue_wo(part):
            per = NWIN // NP
            for br, wo in enumerate((woa, wob)):
                @pl.when(part // (NP // 2) == br)
                def _():
                    def body(i, c):
                        r = pl.multiple_of(((part - br * (NP // 2)) * per + i) * 32, 32)
                        g = br * D + r
                        w_pair((wo, wo), (r, r + 16), (wobuf, wobuf), (g, g + 16),
                               (wosem.at[g // 128], wosem.at[g // 128]))
                        return c
                    lax.fori_loop(0, per, body, 0)

        def issue(step):
            slot = step % NG

            @pl.when(step < NA)
            def _():
                issue_kv(step, slot, ka, va, NCA, 0)

            @pl.when(jnp.logical_and(step >= NA, step < NSTEP))
            def _():
                issue_kv(step - NA, slot, kb, vb, NCB, SK - W)

            @pl.when(jnp.logical_and(step >= NSTEP, step < NSTEP + NP))
            def _():
                issue_wo(step - NSTEP)

        xcp = [pltpu.make_async_copy(x, xbuf.at[i], xsem.at[i]) for i, x in enumerate((xa, xb))]
        for cp, p in zip(xcp, xp):
            cp.start(priority=p)

        def pro_w(i, c):
            r = pl.multiple_of(i * 16, 16)
            w_pair((wqa, wqb), (r, r), (wqbuf.at[0], wqbuf.at[1]), (r, r), (wqsem.at[0], wqsem.at[1]))
            return c
        lax.fori_loop(0, NWIN, pro_w, 0)

        def pro(s, c):
            issue_kv(s, s, ka, va, NCA, 0)
            return c
        lax.fori_loop(0, NG, pro, 0)

        row = lax.broadcasted_iota(jnp.int32, (8, DH), 0)
        even = (row % 2) == 0

        for br in range(2):
            xcp[br].wait()
            xf = xbuf[br].astype(jnp.float32)
            x16 = jnp.concatenate([jnp.broadcast_to(xf[0:1], (8, D)),
                                   jnp.broadcast_to(xf[1:2], (8, D))], axis=0).astype(jnp.bfloat16)
            pltpu.make_async_copy(wqbuf.at[br], wqbuf.at[br], wqsem.at[br]).wait()
            q16 = jnp.dot(x16, wqbuf[br], preferred_element_type=jnp.float32)
            for b in range(B):
                for h in range(HKV):
                    qb = q16[8 * b:8 * b + 8, h * HW:(h + 1) * HW]
                    qbuf[br, b * HKV + h] = jnp.where(even, qb[:, :DH], qb[:, DH:])

        def branch(br, nc, base):
            def segment(seg, c0):
                q8 = qbuf[br, seg].astype(jnp.bfloat16)

                def chunk(c, carry):
                    m, l, acc = carry
                    step = base + seg * nc + c
                    slot = step % NG
                    pltpu.make_async_copy(kvbuf.at[slot, 0], kvbuf.at[slot, 0], kvsem.at[slot, 0]).wait()
                    s = lax.dot_general(q8, kvbuf[slot, 0], (((1,), (1,)), ((), ())),
                                        preferred_element_type=jnp.float32) * (DH ** -0.5)
                    m_new = jnp.maximum(m, jnp.max(s, axis=1, keepdims=True))
                    alpha = jnp.exp(m - m_new)
                    p = jnp.exp(s - m_new)
                    l = alpha * l + jnp.sum(p, axis=1, keepdims=True)
                    pltpu.make_async_copy(kvbuf.at[slot, 1], kvbuf.at[slot, 1], kvsem.at[slot, 1]).wait()
                    acc = alpha * acc + jnp.dot(p.astype(jnp.bfloat16), kvbuf[slot, 1],
                                                preferred_element_type=jnp.float32)
                    issue(step + NG)
                    return m_new, l, acc

                m, l, acc = lax.fori_loop(
                    0, nc, chunk,
                    (jnp.full((8, 1), NEG, jnp.float32), jnp.zeros((8, 1), jnp.float32),
                     jnp.zeros((8, DH), jnp.float32)))
                o8 = acc / l
                obuf[br, seg] = jnp.concatenate([jnp.broadcast_to(o8[0:1], (8, DH)),
                                                 jnp.broadcast_to(o8[1:2], (8, DH))], axis=1)
                return c0
            lax.fori_loop(0, B * HKV, segment, 0)

        branch(0, NCA, 0)
        branch(1, NCB, NA)

        even_w = (lax.broadcasted_iota(jnp.int32, (8, HW), 0) % 2) == 0
        o16 = jnp.concatenate(
            [jnp.concatenate([jnp.where(even_w, obuf[br, h], obuf[br, HKV + h]) for h in range(HKV)], axis=1)
             for br in range(2)], axis=0).astype(jnp.bfloat16)
        lane = lax.broadcasted_iota(jnp.int32, (8, 128), 1)
        for j in range(NOB):
            blk = wobuf.at[pl.ds(j * 128, 128), :]
            pltpu.make_async_copy(blk, blk, wosem.at[j]).wait()
            res = lax.dot_general(o16, blk[...], (((1,), (1,)), ((), ())), preferred_element_type=jnp.float32)
            if (j + 1) * 128 <= D:
                r8 = res[0:8]
            elif j * 128 >= D:
                r8 = res[8:16]
            else:
                r8 = jnp.where(lane < D - j * 128, res[0:8], res[8:16])
            o_ref[:, j * 128:(j + 1) * 128] = r8[0:B].astype(o_ref.dtype)

    @jax.jit
    def f(A_x, A_k_cache, A_v_cache, A_wq, A_wo, B_x, B_k_cache, B_v_cache, B_wq, B_wo):
        out = pl.pallas_call(
            kern,
            in_specs=[pl.BlockSpec(memory_space=pltpu.HBM)] * 10,
            out_specs=pl.BlockSpec(memory_space=pltpu.VMEM),
            out_shape=jax.ShapeDtypeStruct((B, 2 * D), jnp.bfloat16),
            scratch_shapes=[
                pltpu.VMEM((2, B, D), jnp.bfloat16),
                pltpu.VMEM((2, D, HD), jnp.bfloat16),
                pltpu.VMEM((2 * D, HD), jnp.bfloat16),
                pltpu.VMEM((NG, 2, G, DH), jnp.bfloat16),
                pltpu.VMEM((2, B * HKV, 8, DH), jnp.float32),
                pltpu.VMEM((2, B * HKV, 8, HW), jnp.float32),
                pltpu.SemaphoreType.DMA((2,)),
                pltpu.SemaphoreType.DMA((2,)),
                pltpu.SemaphoreType.DMA((NOB,)),
                pltpu.SemaphoreType.DMA((NG, 2)),
            ],
            compiler_params=pltpu.CompilerParams(vmem_limit_bytes=64 * 1024 * 1024, disable_bounds_checks=nobc),
        )(A_x.reshape(B, D), A_k_cache, A_v_cache, A_wq, A_wo.T,
          B_x.reshape(B, D), B_k_cache, B_v_cache, B_wq, B_wo.T)
        return out.reshape(B, 1, 2 * D)
    return f


_impl = make(**dict(nobc=False,G=2048,NG=4))


@jax.jit
def pallas_concat_heads__gqa_block_cached__sliding_block_cached__decode_kernel(
    A_x, A_k_cache, A_v_cache, A_wq, A_wo, B_x, B_k_cache, B_v_cache, B_wq, B_wo
):
    return _impl(A_x, A_k_cache, A_v_cache, A_wq, A_wo, B_x, B_k_cache, B_v_cache, B_wq, B_wo)
```

```python
import numpy as np
import jax
import jax.numpy as jnp
from jax import lax
from jax.experimental import pallas as pl
from jax.experimental.pallas import tpu as pltpu

_HQ, _DH = 16, 256
_CHUNK = 2048
_NSLOT = 3

_KV_PIECES = ((0, 0, 1, 0), (1, 0, 1, 1), (0, 1, 2, 1), (1, 1, 2, 0), (0, 3, 1, 0), (1, 3, 1, 1))
_W_PIECES = ((0, 0, 1, 0), (1, 0, 1, 1), (1, 1, 1, 0), (0, 1, 1, 1),
             (1, 2, 1, 0), (0, 2, 1, 1), (0, 3, 1, 0), (1, 3, 1, 1))
_KV_UNIT = 64

_NT = (((1,), (1,)), ((), ()))


def _kernel(xa, ka, va, wqa, woa, xb, kb, vb, wqb, wob, o_ref,
            xbuf, wqbuf, wobuf, kvbuf, qbuf, obuf, xsem, wqsem, wosem, kvsem,
            *, window, out_groups):
    batch, hkv, sk, dh = ka.shape
    d, hd = wqa.shape
    hw = hd // hkv
    nseg = batch * hkv
    nca, ncb = sk // _CHUNK, window // _CHUNK
    na = nseg * nca
    nstep = na + nseg * ncb

    def fetch_weight_rows(srcs, src_rows, dsts, dst_rows, sem):
        for a, u, _, queue in _W_PIECES:
            r, cols = 8 * (u // 2), pl.ds((hd // 2) * (u % 2), hd // 2)
            pltpu.make_async_copy(srcs[a].at[pl.ds(src_rows[a] + r, 8), cols],
                                  dsts[a].at[pl.ds(dst_rows[a] + r, 8), cols],
                                  sem).start(priority=queue)

    def fetch_kv(j, slot, k, v, nc, first_row):
        seg = j // nc
        b, h = seg // hkv, seg % hkv
        row0 = pl.multiple_of(first_row + (j % nc) * _CHUNK, _CHUNK)
        for w in range(0, _CHUNK, 4 * _KV_UNIT):
            for a, u, n, queue in _KV_PIECES:
                r, nr = w + u * _KV_UNIT, n * _KV_UNIT
                pltpu.make_async_copy((k, v)[a].at[b, h, pl.ds(row0 + r, nr), :],
                                      kvbuf.at[slot, a, pl.ds(r, nr), :],
                                      kvsem.at[slot]).start(priority=queue)

    def fetch_wo(br, wo):
        @pl.loop(0, d // 32)
        def _(i):
            r = pl.multiple_of(i * 32, 32)
            g = br * d + r
            group = sum((g >= e).astype(jnp.int32) for e in out_groups[:-1])
            fetch_weight_rows((wo, wo), (r, r + 16), (wobuf, wobuf), (g, g + 16), wosem.at[group])

    def prefetch(step, br):
        slot = step % _NSLOT
        if br == 0:
            @pl.when(step < na)
            def _():
                fetch_kv(step, slot, ka, va, nca, 0)

        @pl.when(jnp.logical_and(step >= na, step < nstep))
        def _():
            fetch_kv(step - na, slot, kb, vb, ncb, sk - window)

        if br == 1:
            for i, wo in enumerate((woa, wob)):
                @pl.when(step == nstep + i)
                def _():
                    fetch_wo(i, wo)

    x_copies = [pltpu.make_async_copy(x, xbuf.at[i], xsem) for i, x in enumerate((xa, xb))]
    for cp in x_copies:
        cp.start()

    @pl.loop(0, d // 16)
    def _(i):
        r = pl.multiple_of(i * 16, 16)
        fetch_weight_rows((wqa, wqb), (r, r), (wqbuf.at[0], wqbuf.at[1]), (r, r), wqsem)

    @pl.loop(0, _NSLOT)
    def _(s):
        fetch_kv(s, s, ka, va, nca, 0)

    for cp in x_copies:
        cp.wait()
    pltpu.make_async_copy(wqbuf, wqbuf, wqsem).wait()
    even = lax.broadcasted_iota(jnp.int32, (8, dh), 0) % 2 == 0
    for br in range(2):
        x = xbuf[br].astype(jnp.float32)
        x = jnp.concatenate([jnp.broadcast_to(x[b:b + 1], (8, d)) for b in range(batch)], axis=0)
        q = jnp.dot(x.astype(jnp.bfloat16), wqbuf[br], preferred_element_type=jnp.float32)
        for b in range(batch):
            for h in range(hkv):
                qh = q[8 * b:8 * b + 8, h * hw:(h + 1) * hw]
                qbuf[br, b * hkv + h] = jnp.where(even, qh[:, :dh], qh[:, dh:])

    def attend(br, nc, first_step):
        @pl.loop(0, nseg)
        def _(seg):
            q = qbuf[br, seg].astype(jnp.bfloat16)

            def chunk(c, carry):
                m, l, acc = carry
                step = first_step + seg * nc + c
                slot = step % _NSLOT
                pltpu.make_async_copy(kvbuf.at[slot], kvbuf.at[slot], kvsem.at[slot]).wait()
                s = lax.dot_general(q, kvbuf[slot, 0], _NT,
                                    preferred_element_type=jnp.float32) * (dh ** -0.5)
                m_new = jnp.maximum(m, jnp.max(s, axis=1, keepdims=True))
                alpha = jnp.exp(m - m_new)
                p = jnp.exp(s - m_new)
                l = alpha * l + jnp.sum(p, axis=1, keepdims=True)
                acc = alpha * acc + jnp.dot(p.astype(jnp.bfloat16), kvbuf[slot, 1],
                                            preferred_element_type=jnp.float32)
                prefetch(step + _NSLOT, br)
                return m_new, l, acc

            _, l, acc = lax.fori_loop(
                0, nc, chunk,
                (jnp.full((8, 1), float(np.finfo(np.float32).min), jnp.float32),
                 jnp.zeros((8, 1), jnp.float32),
                 jnp.zeros((8, dh), jnp.float32)))
            o = acc / l
            obuf[br, seg] = jnp.concatenate(
                [jnp.broadcast_to(o[g:g + 1], (8, dh)) for g in range(hw // dh)], axis=1)

    attend(0, nca, 0)
    attend(1, ncb, na)

    batch0 = lax.broadcasted_iota(jnp.int32, (8, hw), 0) % 2 == 0
    heads = jnp.concatenate(
        [jnp.concatenate([jnp.where(batch0, obuf[br, h], obuf[br, hkv + h]) for h in range(hkv)], axis=1)
         for br in range(2)], axis=0).astype(jnp.bfloat16)
    for i, (lo, hi) in enumerate(zip((0,) + out_groups[:-1], out_groups)):
        wo = wobuf.at[pl.ds(lo, hi - lo), :]
        pltpu.make_async_copy(wo, wo, wosem.at[i]).wait()
        res = lax.dot_general(heads, wo[...], _NT, preferred_element_type=jnp.float32)
        col = lo + lax.broadcasted_iota(jnp.int32, (8, hi - lo), 1)
        o_ref[:, lo:hi] = jnp.where(col < d, res[0:8], res[8:16])[0:batch].astype(o_ref.dtype)


@jax.jit
def pallas_concat_heads__gqa_block_cached__sliding_block_cached__decode_kernel(
    A_x: jax.Array,
    A_k_cache: jax.Array,
    A_v_cache: jax.Array,
    A_wq: jax.Array,
    A_wo: jax.Array,
    B_x: jax.Array,
    B_k_cache: jax.Array,
    B_v_cache: jax.Array,
    B_wq: jax.Array,
    B_wo: jax.Array,
):
    batch, sq, d = A_x.shape
    _, hkv, sk, dh = A_k_cache.shape
    hd = _HQ * _DH
    window = min(4096, max(256, sk // 4))
    assert (batch, sq, dh, _HQ // hkv) == (2, 1, _DH, 2)
    assert B_k_cache.shape == A_k_cache.shape and B_x.shape == A_x.shape
    assert sk % _CHUNK == 0 and window % _CHUNK == 0 and d % 64 == 0 and d >= 256

    out_groups = tuple(2 * d - 128 * i for i in (3, 2, 1, 0))

    def kernel(*refs):
        _kernel(*refs, window=window, out_groups=out_groups)

    out = pl.pallas_call(
        kernel,
        in_specs=[pl.BlockSpec(memory_space=pltpu.HBM)] * 10,
        out_specs=pl.BlockSpec(memory_space=pltpu.VMEM),
        out_shape=jax.ShapeDtypeStruct((batch, 2 * d), A_x.dtype),
        scratch_shapes=[
            pltpu.VMEM((2, batch, d), A_x.dtype),
            pltpu.VMEM((2, d, hd), A_wq.dtype),
            pltpu.VMEM((2 * d, hd), A_wo.dtype),
            pltpu.VMEM((_NSLOT, 2, _CHUNK, dh), A_k_cache.dtype),
            pltpu.VMEM((2, batch * hkv, 8, dh), jnp.float32),
            pltpu.VMEM((2, batch * hkv, 8, hd // hkv), jnp.float32),
            pltpu.SemaphoreType.DMA(()),
            pltpu.SemaphoreType.DMA(()),
            pltpu.SemaphoreType.DMA((len(out_groups),)),
            pltpu.SemaphoreType.DMA((_NSLOT,)),
        ],
        compiler_params=pltpu.CompilerParams(vmem_limit_bytes=64 * 1024 * 1024),
    )(A_x.reshape(batch, d), A_k_cache, A_v_cache, A_wq, A_wo.T,
      B_x.reshape(batch, d), B_k_cache, B_v_cache, B_wq, B_wo.T)
    return out.reshape(batch, sq, 2 * d)
```
